```python
import jax
import jax.numpy as jnp

def _softmax(x, axis=-1):
    return jax.nn.softmax(x, axis=axis)

def _gelu(x):
    return jax.nn.gelu(x, approximate=True)

def _silu(x):
    return jax.nn.silu(x)

def _sigmoid(x):
    return jax.nn.sigmoid(x)

def _layernorm(x, axis=-1, eps=1e-05):
    m = jnp.mean(x, axis=axis, keepdims=True)
    v = jnp.var(x, axis=axis, keepdims=True)
    return (x - m) / jnp.sqrt(v + eps)

def _scatter_add(tgt, idx, src, axis=0):
    return tgt.at[idx].add(src)

def _segment_sum(src, seg, n):
    return jax.ops.segment_sum(src, seg, n)

class _Rng:

    def __init__(self, key):
        self._k = key

    def _next(self):
        self._k, sub = jax.random.split(self._k)
        return sub

    def normal(self, shape):
        return jax.random.normal(self._next(), shape, dtype=jnp.bfloat16)

    def randint(self, lo, hi, shape):
        return jax.random.randint(self._next(), shape, lo, hi, dtype=jnp.int32)

    def uniform(self, shape, lo=0.0, hi=1.0):
        return jax.random.uniform(self._next(), shape, jnp.bfloat16, lo, hi)

    def permutation(self, n):
        return jax.random.permutation(self._next(), n)
kernel_name = 'adaLN_cond__ssm_conv_h3__dense_activation_gelu__prompt'

def setup_inputs():
    _rng = _Rng(jax.random.key(int.from_bytes(__import__("os").urandom(4), "little")))
    _w = lambda a: (lambda t: t.astype(jnp.bfloat16) if jnp.issubdtype(t.dtype, jnp.floating) else t)(jnp.asarray(a))

    def _A_setup():
        B, S, D = (1, 2048, 640)
        ks = 4
        return {'q': _w((lambda *s: _rng.normal(s) * 0.05)(B, S, D)), 'k': _w((lambda *s: _rng.normal(s) * 0.05)(B, S, D)), 'v': _w((lambda *s: _rng.normal(s) * 0.05)(B, S, D)), 'shift_k': _w((lambda *s: _rng.normal(s) * 0.05)(D, ks) * 0.5), 'ssm_k': _w((lambda *s: _rng.normal(s) * 0.05)(D, S) * (1.0 / S ** 0.5)), 'ssm_D': _w((lambda *s: _rng.normal(s) * 0.05)(D))}
    _A_in = _A_setup()

    def _B_setup():
        B, S, D, F = (1, 2048, 640, 1728)
        return {'x': _w((lambda *s: _rng.normal(s) * 0.05)(B, S, D)), 'w1': _w((lambda *s: _rng.normal(s) * 0.05)(D, F) * D ** (-0.5)), 'b1': _w((lambda *s: _rng.normal(s) * 0.05)(F) * 0.01), 'w2': _w((lambda *s: _rng.normal(s) * 0.05)(F, D) * F ** (-0.5)), 'b2': _w((lambda *s: _rng.normal(s) * 0.05)(D) * 0.01)}
    _B_in = _B_setup()
    return {'A_q': _A_in['q'], 'A_k': _A_in['k'], 'A_v': _A_in['v'], 'A_shift_k': _A_in['shift_k'], 'A_ssm_k': _A_in['ssm_k'], 'A_ssm_D': _A_in['ssm_D'], 'B_x': _B_in['x'], 'B_w1': _B_in['w1'], 'B_b1': _B_in['b1'], 'B_w2': _B_in['w2'], 'B_b2': _B_in['b2'], 'c': _w((lambda *s: _rng.normal(s) * 0.05)(1, 640)), 'w_mod': _w((lambda *s: _rng.normal(s) * 0.05)(640, 6 * 640) * 640 ** (-0.5))}

def reference(A_q, A_k, A_v, A_shift_k, A_ssm_k, A_ssm_D, B_x, B_w1, B_b1, B_w2, B_b2, c, w_mod):

    def _A_ref(q, k, v, shift_k, ssm_k, ssm_D):
        B, S, D = q.shape
        ks = shift_k.shape[-1]
        k_pad = jnp.pad(k, ((0, 0), (ks - 1, 0), (0, 0)))
        k_shift = jnp.zeros_like(k)
        for t in range(ks):
            k_shift = k_shift + k_pad[:, t:t + S, :] * shift_k[:, ks - 1 - t][None, None, :]
        kv = k_shift * v
        L = 2 * S
        kv_pad = jnp.pad(kv, ((0, 0), (0, S), (0, 0)))
        kf_pad = jnp.pad(ssm_k, ((0, 0), (0, S)))
        kv_f = (lambda x, axes=(-2, -1): jnp.fft.rfft2(x.astype(jnp.float32), axes=axes))(kv_pad[:, None, :, :], axes=(1, 2))
        kf_f = (lambda x, axes=(-2, -1): jnp.fft.rfft2(x.astype(jnp.float32), axes=axes))(kf_pad[:, None, :], axes=(1, 2))
        kf_f = (lambda x, *d: x.transpose(*d))(kf_f, 1, 2, 0)
        y_f = kv_f * kf_f[None, :, :, :]
        y = (lambda x, s, axes=(-2, -1): jnp.fft.irfft2(x, s=s, axes=axes).astype(jnp.bfloat16))(y_f, (1, L), axes=(1, 2))[:, 0, :S, :]
        y = y + kv * ssm_D[None, None, :]
        return q * y

    def _B_ref(x, w1, b1, w2, b2):
        h = jnp.einsum('bsd,df->bsf', x, w1) + b1
        h = _gelu(h)
        return jnp.einsum('bsf,fd->bsd', h, w2) + b2
    x = A_q
    mod = (_silu(c) @ w_mod).reshape(c.shape[0], 6, 1, -1)
    sa, ca, ga, sb, cb, gb = (mod[:, 0].copy(), mod[:, 1].copy(), mod[:, 2].copy(), mod[:, 3].copy(), mod[:, 4].copy(), mod[:, 5].copy())
    h = _layernorm(x, axis=-1) * (1 + ca) + sa
    x = x + ga * _A_ref(h, A_k, A_v, A_shift_k, A_ssm_k, A_ssm_D)
    h = _layernorm(x, axis=-1) * (1 + cb) + sb
    x = x + gb * _B_ref(h, B_w1, B_b1, B_w2, B_b2)
    return x
```

```python
import numpy as np
import jax
import jax.numpy as jnp
from jax import lax
import jax.experimental.pallas as pl
import jax.experimental.pallas.tpu as pltpu

S, D, F, KS = 2048, 640, 1728, 4
C = 128
NC = S // C
N = 2 * C
TM = 512
HALO = 16
BF = jnp.bfloat16
F32 = jnp.float32


def _dft_mats():
    f = np.concatenate([np.arange(0, C, 2), np.arange(1, C, 2)]).astype(np.float64)
    w = 2.0 * np.pi * (f + 0.5) / N
    ang = w[:, None] * np.arange(C, dtype=np.float64)[None, :]
    fwd = np.concatenate([np.cos(ang), -np.sin(ang)], axis=0)
    inv = np.concatenate([np.cos(ang).T, -np.sin(ang).T], axis=1) * (2.0 / N)
    return fwd.astype(np.float32), inv.astype(np.float32)


def _ln(x):
    m = jnp.mean(x, axis=-1, keepdims=True)
    xc = x - m
    v = jnp.mean(xc * xc, axis=-1, keepdims=True)
    return xc * lax.rsqrt(v + 1e-5)


def _kernel(q_hbm, k_hbm, v_hbm, sk_hbm, w1_hbm, w2_hbm, wm_hbm,
            shift_ref, ssmd_ref, b1_ref, b2_ref, c_ref, wf_ref, wi_ref,
            o_hbm,
            q_v, k_v, v_v, sk_v, w1_v, w2_v, wm_v, xf, kf, yf, o_v, mod_v, w1t_v,
            sem_in, sem_w, sem_o):
    NG = 4
    GR = S // NG

    def in_copies(g):
        r = pl.ds(g * GR, GR)
        return (
            pltpu.make_async_copy(k_hbm.at[r], k_v.at[pl.ds(HALO + g * GR, GR)], sem_in.at[0, g]),
            pltpu.make_async_copy(v_hbm.at[r], v_v.at[r], sem_in.at[1, g]),
            pltpu.make_async_copy(sk_hbm.at[:, r], sk_v.at[:, r], sem_in.at[2, g]),
        )

    for g in range(2):
        for cp in in_copies(g):
            cp.start()
    cp_wm = pltpu.make_async_copy(wm_hbm, wm_v, sem_w.at[0])
    cp_q = pltpu.make_async_copy(q_hbm, q_v, sem_w.at[1])
    cp_w1 = pltpu.make_async_copy(w1_hbm, w1_v, sem_w.at[2])
    cp_w2 = pltpu.make_async_copy(w2_hbm, w2_v, sem_w.at[3])

    k_v[pl.ds(0, HALO), :] = jnp.zeros((HALO, D), BF)
    kf[0] = jnp.zeros((N, D), F32)
    wf = wf_ref[...]
    shift = shift_ref[...].astype(F32)
    H = C // 2

    for g in range(NG):
        for cp in in_copies(g):
            cp.wait()
        if g + 2 < NG:
            for cp in in_copies(g + 2):
                cp.start()
        elif g + 2 == NG:
            cp_wm.start()
            cp_w1.start()
        else:
            cp_q.start()
            cp_w2.start()

        def p1(i, prev, g=g):
            r0 = pl.multiple_of(i * C, C)
            kk = k_v[pl.ds(r0, C + HALO), :].astype(F32)
            ks = kk[HALO:] * shift[0:1, :]
            for j in range(1, KS):
                ks = ks + pltpu.roll(kk, j, 0)[HALO:] * shift[j:j + 1, :]
            kv = (ks * v_v[pl.ds(r0, C), :].astype(F32)).astype(BF)
            v_v[pl.ds(r0, C), :] = kv
            xf[i] = jnp.dot(wf, kv, preferred_element_type=F32)
            kfi = lax.dot_general(wf, sk_v[:, pl.ds(r0, C)], (((1,), (1,)), ((), ())),
                                  preferred_element_type=F32)
            kc = kf[i] + kfi
            kf[i] = kc

            @pl.when(i + 1 < NC)
            def _():
                kr, ki = kfi[:C], kfi[C:]
                kf[i + 1] = jnp.concatenate(
                    [-ki[:H], ki[H:], kr[:H], -kr[H:]], axis=0)
            return prev

        with jax.named_scope("p1"):
            lax.fori_loop(g * (NC // NG), (g + 1) * (NC // NG), p1, 0)

    def p2(r, carry):
        rr = r * 8
        ri = C + r * 8
        for i in range(NC):
            t1 = t2 = t3 = None
            for j in range(i + 1):
                xr = xf[j, pl.ds(rr, 8), :]
                xi = xf[j, pl.ds(ri, 8), :]
                kr = kf[i - j, pl.ds(rr, 8), :]
                ki = kf[i - j, pl.ds(ri, 8), :]
                p1_ = kr * (xr + xi)
                p2_ = xi * (kr + ki)
                p3_ = xr * (ki - kr)
                t1 = p1_ if t1 is None else t1 + p1_
                t2 = p2_ if t2 is None else t2 + p2_
                t3 = p3_ if t3 is None else t3 + p3_
            yf[i, pl.ds(rr, 8), :] = t1 - t2
            yf[i, pl.ds(ri, 8), :] = t1 + t3
        return carry

    with jax.named_scope("p2"):
        lax.fori_loop(0, C // 8 - 3, p2, 0)

    cp_wm.wait()
    cp_w1.wait()
    for r in range(C // 8 - 3, C // 8):
        p2(r, 0)
    cc = c_ref[...].astype(F32)
    sc = (cc * jax.nn.sigmoid(cc)).astype(BF)
    mod = jnp.dot(jnp.broadcast_to(sc, (8, D)), wm_v[...], preferred_element_type=F32)
    mod_v[...] = mod.astype(BF).astype(F32)
    w1t_v[...] = w1_v[...].T
    cp_q.wait()
    cp_w2.wait()

    def out_copy(t):
        r = pl.ds(pl.multiple_of(t * TM, TM), TM)
        return pltpu.make_async_copy(o_v.at[r], o_hbm.at[r], sem_o.at[t])

    def p3(t, carry):
        r0 = pl.multiple_of(t * TM, TM)
        rows = pl.ds(r0, TM)
        sa, ca, ga = mod_v[0:1, 0:D], mod_v[0:1, D:2 * D], mod_v[0:1, 2 * D:3 * D]
        sb, cb, gb = mod_v[0:1, 3 * D:4 * D], mod_v[0:1, 4 * D:5 * D], mod_v[0:1, 5 * D:6 * D]
        wi = wi_ref[...]
        y = jnp.concatenate(
            [jnp.dot(wi, yf[t * (TM // C) + u].astype(BF), preferred_element_type=F32)
             for u in range(TM // C)], axis=0)
        x = q_v[rows, :].astype(F32)
        kv = v_v[rows, :].astype(F32)
        h = _ln(x) * (1.0 + ca) + sa
        x = x + ga * (h * (y + kv * ssmd_ref[...].astype(F32).reshape(1, D)))
        h2 = (_ln(x) * (1.0 + cb) + sb).astype(BF)
        a = jnp.dot(h2, w1t_v[...], preferred_element_type=F32)
        a = a + b1_ref[...].astype(F32).reshape(1, F)
        a = jax.nn.gelu(a, approximate=True).astype(BF)
        o = jnp.dot(a, w2_v[...], preferred_element_type=F32) + b2_ref[...].astype(F32).reshape(1, D)
        o_v[rows, :] = (x + gb * o).astype(BF)
        out_copy(t).start()
        return carry

    with jax.named_scope("p3"):
        lax.fori_loop(0, S // TM, p3, 0)
    for t in range(S // TM):
        out_copy(t).wait()


@jax.jit
def pallas_adaLN_cond__ssm_conv_h3__dense_activation_gelu__prompt_kernel(
    A_q, A_k, A_v, A_shift_k, A_ssm_k, A_ssm_D, B_x, B_w1, B_b1, B_w2, B_b2, c, w_mod,
):
    del B_x
    wf, wi = _dft_mats()
    any_spec = pl.BlockSpec(memory_space=pl.ANY)
    vm = pl.BlockSpec(memory_space=pltpu.VMEM)
    out = pl.pallas_call(
        _kernel,
        out_shape=jax.ShapeDtypeStruct((S, D), BF),
        in_specs=[any_spec] * 7 + [vm] * 7,
        out_specs=any_spec,
        scratch_shapes=[
            pltpu.VMEM((S, D), BF),
            pltpu.VMEM((S + HALO, D), BF),
            pltpu.VMEM((S, D), BF),
            pltpu.VMEM((D, S), BF),
            pltpu.VMEM((F, D), BF),
            pltpu.VMEM((F, D), BF),
            pltpu.VMEM((D, 6 * D), BF),
            pltpu.VMEM((NC, N, D), F32),
            pltpu.VMEM((NC, N, D), F32),
            pltpu.VMEM((NC, N, D), F32),
            pltpu.VMEM((S, D), BF),
            pltpu.VMEM((8, 6 * D), F32),
            pltpu.VMEM((D, F), BF),
            pltpu.SemaphoreType.DMA((3, 4)),
            pltpu.SemaphoreType.DMA((4,)),
            pltpu.SemaphoreType.DMA((S // TM,)),
        ],
        compiler_params=pltpu.CompilerParams(vmem_limit_bytes=110 * 1024 * 1024),
    )(A_q.reshape(S, D), A_k.reshape(S, D), A_v.reshape(S, D), A_ssm_k, B_w1.T, B_w2, w_mod,
      A_shift_k.T, A_ssm_D, B_b1, B_b2, c,
      jnp.asarray(wf, BF), jnp.asarray(wi, BF))
    return out.reshape(1, S, D)
```

```python
import numpy as np
import jax
import jax.numpy as jnp
from jax import lax
import jax.experimental.pallas as pl
import jax.experimental.pallas.tpu as pltpu

S, D, F, KS = 2048, 640, 1728, 4
C = 128
NC = S // C
N = 2 * C
TM = 512
HALO = 16
BF = jnp.bfloat16
F32 = jnp.float32


def _dft_mats():
    f = np.concatenate([np.arange(0, C, 2), np.arange(1, C, 2)]).astype(np.float64)
    w = 2.0 * np.pi * (f + 0.5) / N
    ang = w[:, None] * np.arange(C, dtype=np.float64)[None, :]
    fwd = np.concatenate([np.cos(ang), -np.sin(ang)], axis=0)
    inv = np.concatenate([np.cos(ang).T, -np.sin(ang).T], axis=1) * (2.0 / N)
    return fwd.astype(np.float32), inv.astype(np.float32)


def _ln(x):
    m = jnp.mean(x, axis=-1, keepdims=True)
    xc = x - m
    v = jnp.mean(xc * xc, axis=-1, keepdims=True)
    return xc * lax.rsqrt(v + 1e-5)


def _kernel(q_hbm, k_hbm, v_hbm, sk_hbm, w1_hbm, w2_hbm, wm_hbm,
            shift_ref, ssmd_ref, b1_ref, b2_ref, c_ref, wf_ref, wi_ref,
            o_hbm,
            q_v, k_v, v_v, sk_v, w1_v, w2_v, wm_v, xf, kf, yf, o_v, mod_v, w1t_v, x_s, h_s,
            sem_in, sem_w, sem_o):
    NG = 4
    GR = S // NG

    def in_copies(g):
        r = pl.ds(g * GR, GR)
        return (
            pltpu.make_async_copy(k_hbm.at[r], k_v.at[pl.ds(HALO + g * GR, GR)], sem_in.at[0, g]),
            pltpu.make_async_copy(v_hbm.at[r], v_v.at[r], sem_in.at[1, g]),
            pltpu.make_async_copy(sk_hbm.at[:, r], sk_v.at[:, r], sem_in.at[2, g]),
        )

    for g in range(2):
        for cp in in_copies(g):
            cp.start()
    cp_wm = pltpu.make_async_copy(wm_hbm, wm_v, sem_w.at[0])
    cp_q = pltpu.make_async_copy(q_hbm, q_v, sem_w.at[1])
    cp_w1 = pltpu.make_async_copy(w1_hbm, w1_v, sem_w.at[2])
    cp_w2 = pltpu.make_async_copy(w2_hbm, w2_v, sem_w.at[3])

    k_v[pl.ds(0, HALO), :] = jnp.zeros((HALO, D), BF)
    kf[0] = jnp.zeros((N, D), F32)
    wf = wf_ref[...]
    shift = shift_ref[...].astype(F32)
    H = C // 2

    for g in range(NG):
        for cp in in_copies(g):
            cp.wait()
        if g + 2 < NG:
            for cp in in_copies(g + 2):
                cp.start()
        elif g + 2 == NG:
            cp_wm.start()
            cp_w1.start()
        else:
            cp_q.start()
            cp_w2.start()

        def p1(i, prev, g=g):
            r0 = pl.multiple_of(i * C, C)
            kk = k_v[pl.ds(r0, C + HALO), :].astype(F32)
            ks = kk[HALO:] * shift[0:1, :]
            for j in range(1, KS):
                ks = ks + pltpu.roll(kk, j, 0)[HALO:] * shift[j:j + 1, :]
            kv = (ks * v_v[pl.ds(r0, C), :].astype(F32)).astype(BF)
            v_v[pl.ds(r0, C), :] = kv
            xf[i] = jnp.dot(wf, kv, preferred_element_type=F32)
            kfi = lax.dot_general(wf, sk_v[:, pl.ds(r0, C)], (((1,), (1,)), ((), ())),
                                  preferred_element_type=F32)
            kc = kf[i] + kfi
            kf[i] = kc

            @pl.when(i + 1 < NC)
            def _():
                kr, ki = kfi[:C], kfi[C:]
                kf[i + 1] = jnp.concatenate(
                    [-ki[:H], ki[H:], kr[:H], -kr[H:]], axis=0)
            return prev

        with jax.named_scope("p1"):
            lax.fori_loop(g * (NC // NG), (g + 1) * (NC // NG), p1, 0)

    def p2(r, carry):
        rr = r * 8
        ri = C + r * 8
        for l in range(D // 128):
            ln = slice(l * 128, (l + 1) * 128)
            xs, ks = [], []
            for j in range(NC):
                xr, xi = xf[j, pl.ds(rr, 8), ln], xf[j, pl.ds(ri, 8), ln]
                kr, ki = kf[j, pl.ds(rr, 8), ln], kf[j, pl.ds(ri, 8), ln]
                xs.append((xr + xi, xi, xr))
                ks.append((kr, kr + ki, ki - kr))
            acc = []
            for p in range(3):
                for i in range(NC):
                    t = xs[0][p] * ks[i][p]
                    for j in range(1, i + 1):
                        t = t + xs[j][p] * ks[i - j][p]
                    acc.append(t)
            for i in range(NC):
                yf[i, pl.ds(rr, 8), ln] = acc[i] - acc[NC + i]
                yf[i, pl.ds(ri, 8), ln] = acc[i] + acc[2 * NC + i]
        return carry

    with jax.named_scope("p2"):
        lax.fori_loop(0, C // 8 - 3, p2, 0)

    cp_wm.wait()
    cp_w1.wait()
    for r in range(C // 8 - 3, C // 8):
        p2(r, 0)
    cc = c_ref[...].astype(F32)
    sc = (cc * jax.nn.sigmoid(cc)).astype(BF)
    mod = jnp.dot(jnp.broadcast_to(sc, (8, D)), wm_v[...], preferred_element_type=F32)
    mod_v[...] = mod.astype(BF).astype(F32)
    w1t_v[...] = w1_v[...].T
    cp_q.wait()
    cp_w2.wait()

    def out_copy(t):
        r = pl.ds(pl.multiple_of(t * TM, TM), TM)
        return pltpu.make_async_copy(o_v.at[r], o_hbm.at[r], sem_o.at[t])

    def p3(t, carry):
        r0 = pl.multiple_of(t * TM, TM)
        rows = pl.ds(r0, TM)
        sa, ca, ga = mod_v[0:1, 0:D], mod_v[0:1, D:2 * D], mod_v[0:1, 2 * D:3 * D]
        sb, cb, gb = mod_v[0:1, 3 * D:4 * D], mod_v[0:1, 4 * D:5 * D], mod_v[0:1, 5 * D:6 * D]
        wi = wi_ref[...]
        sd = ssmd_ref[...].astype(F32).reshape(1, D)
        for u in range(TM // C):
            i = t * (TM // C) + u
            y = jnp.dot(wi, yf[i].astype(BF), preferred_element_type=F32)
            for b in range(C // 16):
                l0 = u * C + b * 16
                rr = pl.ds(r0 + l0, 16)
                x = q_v[rr, :].astype(F32)
                kv = v_v[rr, :].astype(F32)
                h = _ln(x) * (1.0 + ca) + sa
                x = x + ga * (h * (y[b * 16:b * 16 + 16] + kv * sd))
                x_s[l0:l0 + 16, :] = x
                h_s[l0:l0 + 16, :] = (_ln(x) * (1.0 + cb) + sb).astype(BF)
        h2 = h_s[...]
        x = x_s[...]
        a = jnp.dot(h2, w1t_v[...], preferred_element_type=F32)
        a = a + b1_ref[...].astype(F32).reshape(1, F)
        a = jax.nn.gelu(a, approximate=True).astype(BF)
        o = jnp.dot(a, w2_v[...], preferred_element_type=F32) + b2_ref[...].astype(F32).reshape(1, D)
        o_v[rows, :] = (x + gb * o).astype(BF)
        out_copy(t).start()
        return carry

    with jax.named_scope("p3"):
        lax.fori_loop(0, S // TM, p3, 0)
    for t in range(S // TM):
        out_copy(t).wait()


@jax.jit
def pallas_adaLN_cond__ssm_conv_h3__dense_activation_gelu__prompt_kernel(
    A_q, A_k, A_v, A_shift_k, A_ssm_k, A_ssm_D, B_x, B_w1, B_b1, B_w2, B_b2, c, w_mod,
):
    del B_x
    wf, wi = _dft_mats()
    any_spec = pl.BlockSpec(memory_space=pl.ANY)
    vm = pl.BlockSpec(memory_space=pltpu.VMEM)
    out = pl.pallas_call(
        _kernel,
        out_shape=jax.ShapeDtypeStruct((S, D), BF),
        in_specs=[any_spec] * 7 + [vm] * 7,
        out_specs=any_spec,
        scratch_shapes=[
            pltpu.VMEM((S, D), BF),
            pltpu.VMEM((S + HALO, D), BF),
            pltpu.VMEM((S, D), BF),
            pltpu.VMEM((D, S), BF),
            pltpu.VMEM((F, D), BF),
            pltpu.VMEM((F, D), BF),
            pltpu.VMEM((D, 6 * D), BF),
            pltpu.VMEM((NC, N, D), F32),
            pltpu.VMEM((NC, N, D), F32),
            pltpu.VMEM((NC, N, D), F32),
            pltpu.VMEM((S, D), BF),
            pltpu.VMEM((8, 6 * D), F32),
            pltpu.VMEM((D, F), BF),
            pltpu.VMEM((TM, D), F32),
            pltpu.VMEM((TM, D), BF),
            pltpu.SemaphoreType.DMA((3, 4)),
            pltpu.SemaphoreType.DMA((4,)),
            pltpu.SemaphoreType.DMA((S // TM,)),
        ],
        compiler_params=pltpu.CompilerParams(vmem_limit_bytes=110 * 1024 * 1024),
    )(A_q.reshape(S, D), A_k.reshape(S, D), A_v.reshape(S, D), A_ssm_k, B_w1.T, B_w2, w_mod,
      A_shift_k.T, A_ssm_D, B_b1, B_b2, c,
      jnp.asarray(wf, BF), jnp.asarray(wi, BF))
    return out.reshape(1, S, D)
```

```python
import numpy as np
import jax
import jax.numpy as jnp
from jax import lax
import jax.experimental.pallas as pl
import jax.experimental.pallas.tpu as pltpu

S, D, F, KS = 2048, 640, 1728, 4
C = 128
NC = S // C
N = 2 * C
TM = 512
HALO = 16
BF = jnp.bfloat16
F32 = jnp.float32


def _dft_mats():
    f = np.concatenate([np.arange(0, C, 2), np.arange(1, C, 2)]).astype(np.float64)
    w = 2.0 * np.pi * (f + 0.5) / N
    ang = w[:, None] * np.arange(C, dtype=np.float64)[None, :]
    fwd = np.concatenate([np.cos(ang), -np.sin(ang)], axis=0)
    inv = np.concatenate([np.cos(ang).T, -np.sin(ang).T], axis=1) * (2.0 / N)
    return fwd.astype(np.float32), inv.astype(np.float32)


def _ln(x):
    m = jnp.mean(x, axis=-1, keepdims=True)
    xc = x - m
    v = jnp.mean(xc * xc, axis=-1, keepdims=True)
    return xc * lax.rsqrt(v + 1e-5)


def _kernel(q_hbm, k_hbm, v_hbm, sk_hbm, w1_hbm, w2_hbm, wm_hbm,
            shift_ref, ssmd_ref, b1_ref, b2_ref, c_ref, wf_ref, wi_ref,
            o_hbm,
            q_v, k_v, v_v, sk_v, w1_v, w2_v, wm_v, xf, kf, yf, o_v, mod_v, w1t_v, x_s, h_s,
            sem_in, sem_w, sem_o):
    NG = 4
    GR = S // NG

    def in_copies(g):
        r = pl.ds(g * GR, GR)
        return (
            pltpu.make_async_copy(k_hbm.at[r], k_v.at[pl.ds(HALO + g * GR, GR)], sem_in.at[0, g]),
            pltpu.make_async_copy(v_hbm.at[r], v_v.at[r], sem_in.at[1, g]),
            pltpu.make_async_copy(sk_hbm.at[:, r], sk_v.at[:, r], sem_in.at[2, g]),
        )

    for g in range(2):
        for cp in in_copies(g):
            cp.start()
    cp_wm = pltpu.make_async_copy(wm_hbm, wm_v, sem_w.at[0])
    cp_q = pltpu.make_async_copy(q_hbm, q_v, sem_w.at[1])
    cp_w1 = pltpu.make_async_copy(w1_hbm, w1_v, sem_w.at[2])
    cp_w2 = pltpu.make_async_copy(w2_hbm, w2_v, sem_w.at[3])

    k_v[pl.ds(0, HALO), :] = jnp.zeros((HALO, D), BF)
    kf[0] = jnp.zeros((N, D), F32)
    wf = wf_ref[...]
    shift = shift_ref[...].astype(F32)
    H = C // 2

    for g in range(NG):
        for cp in in_copies(g):
            cp.wait()
        if g + 2 < NG:
            for cp in in_copies(g + 2):
                cp.start()
        elif g + 2 == NG:
            cp_wm.start()
            cp_w1.start()
        else:
            cp_q.start()
            cp_w2.start()

        def p1(i, prev, g=g):
            r0 = pl.multiple_of(i * C, C)
            kk = k_v[pl.ds(r0, C + HALO), :].astype(F32)
            ks = kk[HALO:] * shift[0:1, :]
            for j in range(1, KS):
                ks = ks + pltpu.roll(kk, j, 0)[HALO:] * shift[j:j + 1, :]
            kv = (ks * v_v[pl.ds(r0, C), :].astype(F32)).astype(BF)
            v_v[pl.ds(r0, C), :] = kv
            xf[i] = jnp.dot(wf, kv, preferred_element_type=F32)
            kfi = lax.dot_general(wf, sk_v[:, pl.ds(r0, C)], (((1,), (1,)), ((), ())),
                                  preferred_element_type=F32)
            kc = kf[i] + kfi
            kf[i] = kc

            @pl.when(i + 1 < NC)
            def _():
                kr, ki = kfi[:C], kfi[C:]
                kf[i + 1] = jnp.concatenate(
                    [-ki[:H], ki[H:], kr[:H], -kr[H:]], axis=0)
            return prev

        with jax.named_scope("p1"):
            lax.fori_loop(g * (NC // NG), (g + 1) * (NC // NG), p1, 0)

    def p2(r, carry):
        rr = r * 8
        ri = C + r * 8
        for l in range(D // 128):
            ln = slice(l * 128, (l + 1) * 128)
            A, B = pl.ds(rr, 8), pl.ds(ri, 8)
            for p in range(3):
                if p == 0:
                    xs = [xf[j, A, ln] + xf[j, B, ln] for j in range(NC)]
                    ks = [kf[j, A, ln] for j in range(NC)]
                elif p == 1:
                    xs = [xf[j, B, ln] for j in range(NC)]
                    ks = [kf[j, A, ln] + kf[j, B, ln] for j in range(NC)]
                else:
                    xs = [xf[j, A, ln] for j in range(NC)]
                    ks = [kf[j, B, ln] - kf[j, A, ln] for j in range(NC)]
                for i in range(NC):
                    t = xs[0] * ks[i]
                    for j in range(1, i + 1):
                        t = t + xs[j] * ks[i - j]
                    if p == 0:
                        yf[i, A, ln] = t
                        yf[i, B, ln] = t
                    elif p == 1:
                        yf[i, A, ln] = yf[i, A, ln] - t
                    else:
                        yf[i, B, ln] = yf[i, B, ln] + t
        return carry

    with jax.named_scope("p2"):
        lax.fori_loop(0, C // 8 - 3, p2, 0)

    cp_wm.wait()
    cp_w1.wait()
    for r in range(C // 8 - 3, C // 8):
        p2(r, 0)
    cc = c_ref[...].astype(F32)
    sc = (cc * jax.nn.sigmoid(cc)).astype(BF)
    mod = jnp.dot(jnp.broadcast_to(sc, (8, D)), wm_v[...], preferred_element_type=F32)
    mod_v[...] = mod.astype(BF).astype(F32)
    w1t_v[...] = w1_v[...].T
    cp_q.wait()
    cp_w2.wait()

    def out_copy(t):
        r = pl.ds(pl.multiple_of(t * TM, TM), TM)
        return pltpu.make_async_copy(o_v.at[r], o_hbm.at[r], sem_o.at[t])

    def p3(t, carry):
        r0 = pl.multiple_of(t * TM, TM)
        rows = pl.ds(r0, TM)
        sa, ca, ga = mod_v[0:1, 0:D], mod_v[0:1, D:2 * D], mod_v[0:1, 2 * D:3 * D]
        sb, cb, gb = mod_v[0:1, 3 * D:4 * D], mod_v[0:1, 4 * D:5 * D], mod_v[0:1, 5 * D:6 * D]
        wi = wi_ref[...]
        sd = ssmd_ref[...].astype(F32).reshape(1, D)
        for u in range(TM // C):
            i = t * (TM // C) + u
            y = jnp.dot(wi, yf[i].astype(BF), preferred_element_type=F32)
            for b in range(C // 16):
                l0 = u * C + b * 16
                rr = pl.ds(r0 + l0, 16)
                x = q_v[rr, :].astype(F32)
                kv = v_v[rr, :].astype(F32)
                h = _ln(x) * (1.0 + ca) + sa
                x = x + ga * (h * (y[b * 16:b * 16 + 16] + kv * sd))
                x_s[l0:l0 + 16, :] = x
                h_s[l0:l0 + 16, :] = (_ln(x) * (1.0 + cb) + sb).astype(BF)
        h2 = h_s[...]
        x = x_s[...]
        a = jnp.dot(h2, w1t_v[...], preferred_element_type=F32)
        a = a + b1_ref[...].astype(F32).reshape(1, F)
        a = jax.nn.gelu(a, approximate=True).astype(BF)
        o = jnp.dot(a, w2_v[...], preferred_element_type=F32) + b2_ref[...].astype(F32).reshape(1, D)
        o_v[rows, :] = (x + gb * o).astype(BF)
        out_copy(t).start()
        return carry

    with jax.named_scope("p3"):
        lax.fori_loop(0, S // TM, p3, 0)
    for t in range(S // TM):
        out_copy(t).wait()


@jax.jit
def pallas_adaLN_cond__ssm_conv_h3__dense_activation_gelu__prompt_kernel(
    A_q, A_k, A_v, A_shift_k, A_ssm_k, A_ssm_D, B_x, B_w1, B_b1, B_w2, B_b2, c, w_mod,
):
    del B_x
    wf, wi = _dft_mats()
    any_spec = pl.BlockSpec(memory_space=pl.ANY)
    vm = pl.BlockSpec(memory_space=pltpu.VMEM)
    out = pl.pallas_call(
        _kernel,
        out_shape=jax.ShapeDtypeStruct((S, D), BF),
        in_specs=[any_spec] * 7 + [vm] * 7,
        out_specs=any_spec,
        scratch_shapes=[
            pltpu.VMEM((S, D), BF),
            pltpu.VMEM((S + HALO, D), BF),
            pltpu.VMEM((S, D), BF),
            pltpu.VMEM((D, S), BF),
            pltpu.VMEM((F, D), BF),
            pltpu.VMEM((F, D), BF),
            pltpu.VMEM((D, 6 * D), BF),
            pltpu.VMEM((NC, N, D), F32),
            pltpu.VMEM((NC, N, D), F32),
            pltpu.VMEM((NC, N, D), F32),
            pltpu.VMEM((S, D), BF),
            pltpu.VMEM((8, 6 * D), F32),
            pltpu.VMEM((D, F), BF),
            pltpu.VMEM((TM, D), F32),
            pltpu.VMEM((TM, D), BF),
            pltpu.SemaphoreType.DMA((3, 4)),
            pltpu.SemaphoreType.DMA((4,)),
            pltpu.SemaphoreType.DMA((S // TM,)),
        ],
        compiler_params=pltpu.CompilerParams(vmem_limit_bytes=110 * 1024 * 1024),
    )(A_q.reshape(S, D), A_k.reshape(S, D), A_v.reshape(S, D), A_ssm_k, B_w1.T, B_w2, w_mod,
      A_shift_k.T, A_ssm_D, B_b1, B_b2, c,
      jnp.asarray(wf, BF), jnp.asarray(wi, BF))
    return out.reshape(1, S, D)
```

```python
import numpy as np
import jax
import jax.numpy as jnp
from jax import lax
import jax.experimental.pallas as pl
import jax.experimental.pallas.tpu as pltpu

S, D, F, KS = 2048, 640, 1728, 4
C = 128
NC = S // C
N = 2 * C
TM = 256
HALO = 16
BF = jnp.bfloat16
F32 = jnp.float32


def _dft_mats():
    f = np.concatenate([np.arange(0, C, 2), np.arange(1, C, 2)]).astype(np.float64)
    w = 2.0 * np.pi * (f + 0.5) / N
    ang = w[:, None] * np.arange(C, dtype=np.float64)[None, :]
    fwd = np.concatenate([np.cos(ang), -np.sin(ang)], axis=0)
    inv = np.concatenate([np.cos(ang).T, -np.sin(ang).T], axis=1) * (2.0 / N)
    return fwd.astype(np.float32), inv.astype(np.float32)


def _ln(x):
    m = jnp.mean(x, axis=-1, keepdims=True)
    xc = x - m
    v = jnp.mean(xc * xc, axis=-1, keepdims=True)
    return xc * lax.rsqrt(v + 1e-5)


def _kernel(q_hbm, k_hbm, v_hbm, sk_hbm, w1_hbm, w2_hbm, wm_hbm,
            shift_ref, ssmd_ref, b1_ref, b2_ref, c_ref, wf_ref, wi_ref,
            o_hbm,
            q_v, k_v, v_v, sk_v, w1_v, w2_v, wm_v, xf, kf, yf, o_v, mod_v, w1t_v, x_s, h_s, x_t, h_t,
            sem_in, sem_w, sem_o):
    NG = 4
    GR = S // NG

    def in_copies(g):
        r = pl.ds(g * GR, GR)
        return (
            pltpu.make_async_copy(k_hbm.at[r], k_v.at[pl.ds(HALO + g * GR, GR)], sem_in.at[0, g]),
            pltpu.make_async_copy(v_hbm.at[r], v_v.at[r], sem_in.at[1, g]),
            pltpu.make_async_copy(sk_hbm.at[:, r], sk_v.at[:, r], sem_in.at[2, g]),
        )

    for g in range(2):
        for cp in in_copies(g):
            cp.start()
    cp_wm = pltpu.make_async_copy(wm_hbm, wm_v, sem_w.at[0])
    cp_q = pltpu.make_async_copy(q_hbm, q_v, sem_w.at[1])
    cp_w1 = pltpu.make_async_copy(w1_hbm, w1_v, sem_w.at[2])
    cp_w2 = pltpu.make_async_copy(w2_hbm, w2_v, sem_w.at[3])

    k_v[pl.ds(0, HALO), :] = jnp.zeros((HALO, D), BF)
    kf[0] = jnp.zeros((N, D), F32)
    wf = wf_ref[...]
    shift = shift_ref[...].astype(F32)
    H = C // 2

    for g in range(NG):
        for cp in in_copies(g):
            cp.wait()
        if g + 2 < NG:
            for cp in in_copies(g + 2):
                cp.start()
        elif g + 2 == NG:
            cp_wm.start()
            cp_w1.start()
        else:
            cp_q.start()
            cp_w2.start()

        def p1(i, prev, g=g):
            r0 = pl.multiple_of(i * C, C)
            kk = k_v[pl.ds(r0, C + HALO), :].astype(F32)
            ks = kk[HALO:] * shift[0:1, :]
            for j in range(1, KS):
                ks = ks + pltpu.roll(kk, j, 0)[HALO:] * shift[j:j + 1, :]
            kv = (ks * v_v[pl.ds(r0, C), :].astype(F32)).astype(BF)
            v_v[pl.ds(r0, C), :] = kv
            xf[i] = jnp.dot(wf, kv, preferred_element_type=F32)
            kfi = lax.dot_general(wf, sk_v[:, pl.ds(r0, C)], (((1,), (1,)), ((), ())),
                                  preferred_element_type=F32)
            kc = kf[i] + kfi
            kf[i] = kc

            @pl.when(i + 1 < NC)
            def _():
                kr, ki = kfi[:C], kfi[C:]
                kf[i + 1] = jnp.concatenate(
                    [-ki[:H], ki[H:], kr[:H], -kr[H:]], axis=0)
            return prev

        with jax.named_scope("p1"):
            lax.fori_loop(g * (NC // NG), (g + 1) * (NC // NG), p1, 0)

    def p2(r, carry):
        rr = r * 8
        ri = C + r * 8
        for l in range(D // 128):
            ln = slice(l * 128, (l + 1) * 128)
            A, B = pl.ds(rr, 8), pl.ds(ri, 8)
            for p in range(3):
                if p == 0:
                    xs = [xf[j, A, ln] + xf[j, B, ln] for j in range(NC)]
                    ks = [kf[j, A, ln] for j in range(NC)]
                elif p == 1:
                    xs = [xf[j, B, ln] for j in range(NC)]
                    ks = [kf[j, A, ln] + kf[j, B, ln] for j in range(NC)]
                else:
                    xs = [xf[j, A, ln] for j in range(NC)]
                    ks = [kf[j, B, ln] - kf[j, A, ln] for j in range(NC)]
                for i in range(NC):
                    t = xs[0] * ks[i]
                    for j in range(1, i + 1):
                        t = t + xs[j] * ks[i - j]
                    if p == 0:
                        yf[i, A, ln] = t
                        yf[i, B, ln] = t
                    elif p == 1:
                        yf[i, A, ln] = yf[i, A, ln] - t
                    else:
                        yf[i, B, ln] = yf[i, B, ln] + t
        return carry

    with jax.named_scope("p2"):
        lax.fori_loop(0, C // 8 - 3, p2, 0)

    cp_wm.wait()
    cp_w1.wait()
    for r in range(C // 8 - 3, C // 8):
        p2(r, 0)
    cc = c_ref[...].astype(F32)
    sc = (cc * jax.nn.sigmoid(cc)).astype(BF)
    mod = jnp.dot(jnp.broadcast_to(sc, (8, D)), wm_v[...], preferred_element_type=F32)
    mod_v[...] = mod.astype(BF).astype(F32)
    w1t_v[...] = w1_v[...].T
    cp_q.wait()
    cp_w2.wait()

    def out_copy(t):
        r = pl.ds(pl.multiple_of(t * TM, TM), TM)
        return pltpu.make_async_copy(o_v.at[r], o_hbm.at[r], sem_o.at[t])

    def pre(t, x_s, h_s):
        r0 = pl.multiple_of(t * TM, TM)
        rows = pl.ds(r0, TM)
        sa, ca, ga = mod_v[0:1, 0:D], mod_v[0:1, D:2 * D], mod_v[0:1, 2 * D:3 * D]
        sb, cb, gb = mod_v[0:1, 3 * D:4 * D], mod_v[0:1, 4 * D:5 * D], mod_v[0:1, 5 * D:6 * D]
        wi = wi_ref[...]
        sd = ssmd_ref[...].astype(F32).reshape(1, D)
        for u in range(TM // C):
            i = t * (TM // C) + u
            y = jnp.dot(wi, yf[i].astype(BF), preferred_element_type=F32)
            for b in range(C // 16):
                l0 = u * C + b * 16
                rr = pl.ds(r0 + l0, 16)
                x = q_v[rr, :].astype(F32)
                kv = v_v[rr, :].astype(F32)
                h = _ln(x) * (1.0 + ca) + sa
                x = x + ga * (h * (y[b * 16:b * 16 + 16] + kv * sd))
                x_s[l0:l0 + 16, :] = x
                h_s[l0:l0 + 16, :] = (_ln(x) * (1.0 + cb) + sb).astype(BF)

    def ffn(t, x_s, h_s):
        rows = pl.ds(pl.multiple_of(t * TM, TM), TM)
        gb = mod_v[0:1, 5 * D:6 * D]
        h2 = h_s[...]
        x = x_s[...]
        a = jnp.dot(h2, w1t_v[...], preferred_element_type=F32)
        a = a + b1_ref[...].astype(F32).reshape(1, F)
        a = jax.nn.gelu(a, approximate=True).astype(BF)
        o = jnp.dot(a, w2_v[...], preferred_element_type=F32) + b2_ref[...].astype(F32).reshape(1, D)
        o_v[rows, :] = (x + gb * o).astype(BF)

    def p3(u, carry):
        t = 2 * u
        pre(t + 1, x_t, h_t)
        ffn(t, x_s, h_s)
        pre(jnp.minimum(t + 2, S // TM - 1), x_s, h_s)
        ffn(t + 1, x_t, h_t)
        out_copy(t).start()
        out_copy(t + 1).start()
        return carry

    with jax.named_scope("p3"):
        pre(0, x_s, h_s)
        lax.fori_loop(0, S // TM // 2, p3, 0)
    for t in range(S // TM):
        out_copy(t).wait()


@jax.jit
def pallas_adaLN_cond__ssm_conv_h3__dense_activation_gelu__prompt_kernel(
    A_q, A_k, A_v, A_shift_k, A_ssm_k, A_ssm_D, B_x, B_w1, B_b1, B_w2, B_b2, c, w_mod,
):
    del B_x
    wf, wi = _dft_mats()
    any_spec = pl.BlockSpec(memory_space=pl.ANY)
    vm = pl.BlockSpec(memory_space=pltpu.VMEM)
    out = pl.pallas_call(
        _kernel,
        out_shape=jax.ShapeDtypeStruct((S, D), BF),
        in_specs=[any_spec] * 7 + [vm] * 7,
        out_specs=any_spec,
        scratch_shapes=[
            pltpu.VMEM((S, D), BF),
            pltpu.VMEM((S + HALO, D), BF),
            pltpu.VMEM((S, D), BF),
            pltpu.VMEM((D, S), BF),
            pltpu.VMEM((F, D), BF),
            pltpu.VMEM((F, D), BF),
            pltpu.VMEM((D, 6 * D), BF),
            pltpu.VMEM((NC, N, D), F32),
            pltpu.VMEM((NC, N, D), F32),
            pltpu.VMEM((NC, N, D), F32),
            pltpu.VMEM((S, D), BF),
            pltpu.VMEM((8, 6 * D), F32),
            pltpu.VMEM((D, F), BF),
            pltpu.VMEM((TM, D), F32),
            pltpu.VMEM((TM, D), BF),
            pltpu.VMEM((TM, D), F32),
            pltpu.VMEM((TM, D), BF),
            pltpu.SemaphoreType.DMA((3, 4)),
            pltpu.SemaphoreType.DMA((4,)),
            pltpu.SemaphoreType.DMA((S // TM,)),
        ],
        compiler_params=pltpu.CompilerParams(vmem_limit_bytes=110 * 1024 * 1024),
    )(A_q.reshape(S, D), A_k.reshape(S, D), A_v.reshape(S, D), A_ssm_k, B_w1.T, B_w2, w_mod,
      A_shift_k.T, A_ssm_D, B_b1, B_b2, c,
      jnp.asarray(wf, BF), jnp.asarray(wi, BF))
    return out.reshape(1, S, D)
```

```python
import numpy as np
import jax
import jax.numpy as jnp
from jax import lax
import jax.experimental.pallas as pl
import jax.experimental.pallas.tpu as pltpu

S, D, F, KS = 2048, 640, 1728, 4
C = 128
NC = S // C
N = 2 * C
TM = 256
HALO = 16
BF = jnp.bfloat16
F32 = jnp.float32


def _dft_mats():
    f = np.concatenate([np.arange(0, C, 2), np.arange(1, C, 2)]).astype(np.float64)
    w = 2.0 * np.pi * (f + 0.5) / N
    ang = w[:, None] * np.arange(C, dtype=np.float64)[None, :]
    fwd = np.concatenate([np.cos(ang), -np.sin(ang)], axis=0)
    inv = np.concatenate([np.cos(ang).T, -np.sin(ang).T], axis=1) * (2.0 / N)
    return fwd.astype(np.float32), inv.astype(np.float32)


def _ln(x):
    m = jnp.mean(x, axis=-1, keepdims=True)
    xc = x - m
    v = jnp.mean(xc * xc, axis=-1, keepdims=True)
    return xc * lax.rsqrt(v + 1e-5)


def _kernel(q_hbm, k_hbm, v_hbm, sk_hbm, w1_hbm, w2_hbm, wm_hbm,
            shift_ref, ssmd_ref, b1_ref, b2_ref, c_ref, wf_ref, wi_ref,
            o_hbm,
            q_v, k_v, v_v, sk_v, w1_v, w2_v, wm_v, xf, kf, yf, o_v, mod_v, w1t_v, x_s, h_s, x_t, h_t,
            sem_in, sem_w, sem_o):
    NG = 4
    GR = S // NG

    def in_copies(g):
        r = pl.ds(g * GR, GR)
        return (
            pltpu.make_async_copy(k_hbm.at[r], k_v.at[pl.ds(HALO + g * GR, GR)], sem_in.at[0, g]),
            pltpu.make_async_copy(v_hbm.at[r], v_v.at[r], sem_in.at[1, g]),
            pltpu.make_async_copy(sk_hbm.at[:, r], sk_v.at[:, r], sem_in.at[2, g]),
        )

    for g in range(2):
        for cp in in_copies(g):
            cp.start()
    cp_wm = pltpu.make_async_copy(wm_hbm, wm_v, sem_w.at[0])
    cp_q = pltpu.make_async_copy(q_hbm, q_v, sem_w.at[1])
    cp_w1 = pltpu.make_async_copy(w1_hbm, w1_v, sem_w.at[2])
    cp_w2 = pltpu.make_async_copy(w2_hbm, w2_v, sem_w.at[3])

    k_v[pl.ds(0, HALO), :] = jnp.zeros((HALO, D), BF)
    kf[0] = jnp.zeros((N, D), F32)
    wf = wf_ref[...]
    shift = shift_ref[...].astype(F32)
    H = C // 2

    for g in range(NG):
        for cp in in_copies(g):
            cp.wait()
        if g + 2 < NG:
            for cp in in_copies(g + 2):
                cp.start()
        elif g + 2 == NG:
            cp_wm.start()
            cp_w1.start()
        else:
            cp_q.start()
            cp_w2.start()

        def p1(i, prev, g=g):
            r0 = pl.multiple_of(i * C, C)
            kk = k_v[pl.ds(r0, C + HALO), :].astype(F32)
            ks = kk[HALO:] * shift[0:1, :]
            for j in range(1, KS):
                ks = ks + pltpu.roll(kk, j, 0)[HALO:] * shift[j:j + 1, :]
            kv = (ks * v_v[pl.ds(r0, C), :].astype(F32)).astype(BF)
            v_v[pl.ds(r0, C), :] = kv
            xf[i] = jnp.dot(wf, kv, preferred_element_type=F32)
            kfi = lax.dot_general(wf, sk_v[:, pl.ds(r0, C)], (((1,), (1,)), ((), ())),
                                  preferred_element_type=F32)
            kc = kf[i] + kfi
            kf[i] = kc

            kr, ki = kfi[:C], kfi[C:]
            kf[i + 1] = jnp.concatenate(
                [-ki[:H], ki[H:], kr[:H], -kr[H:]], axis=0)
            return prev

        with jax.named_scope("p1"):
            lax.fori_loop(g * (NC // NG), (g + 1) * (NC // NG), p1, 0, unroll=2)

    def p2(r, carry):
        rr = r * 8
        ri = C + r * 8
        for l in range(D // 128):
            ln = slice(l * 128, (l + 1) * 128)
            A, B = pl.ds(rr, 8), pl.ds(ri, 8)
            for p in range(3):
                if p == 0:
                    xs = [xf[j, A, ln] + xf[j, B, ln] for j in range(NC)]
                    ks = [kf[j, A, ln] for j in range(NC)]
                elif p == 1:
                    xs = [xf[j, B, ln] for j in range(NC)]
                    ks = [kf[j, A, ln] + kf[j, B, ln] for j in range(NC)]
                else:
                    xs = [xf[j, A, ln] for j in range(NC)]
                    ks = [kf[j, B, ln] - kf[j, A, ln] for j in range(NC)]
                for i in range(NC):
                    t = xs[0] * ks[i]
                    for j in range(1, i + 1):
                        t = t + xs[j] * ks[i - j]
                    if p == 0:
                        yf[i, A, ln] = t
                        yf[i, B, ln] = t
                    elif p == 1:
                        yf[i, A, ln] = yf[i, A, ln] - t
                    else:
                        yf[i, B, ln] = yf[i, B, ln] + t
        return carry

    with jax.named_scope("p2"):
        lax.fori_loop(0, C // 8 - 3, p2, 0)

    cp_wm.wait()
    cp_w1.wait()
    for r in range(C // 8 - 3, C // 8):
        p2(r, 0)
    cc = c_ref[...].astype(F32)
    sc = (cc * jax.nn.sigmoid(cc)).astype(BF)
    mod = jnp.dot(jnp.broadcast_to(sc, (8, D)), wm_v[...], preferred_element_type=F32)
    mod_v[...] = mod.astype(BF).astype(F32)
    w1t_v[...] = w1_v[...].T
    cp_q.wait()
    cp_w2.wait()

    def out_copy(t):
        r = pl.ds(pl.multiple_of(t * TM, TM), TM)
        return pltpu.make_async_copy(o_v.at[r], o_hbm.at[r], sem_o.at[t])

    def pre(t, x_s, h_s):
        r0 = pl.multiple_of(t * TM, TM)
        rows = pl.ds(r0, TM)
        sa, ca, ga = mod_v[0:1, 0:D], mod_v[0:1, D:2 * D], mod_v[0:1, 2 * D:3 * D]
        sb, cb, gb = mod_v[0:1, 3 * D:4 * D], mod_v[0:1, 4 * D:5 * D], mod_v[0:1, 5 * D:6 * D]
        wi = wi_ref[...]
        sd = ssmd_ref[...].astype(F32).reshape(1, D)
        for u in range(TM // C):
            i = t * (TM // C) + u
            y = jnp.dot(wi, yf[i].astype(BF), preferred_element_type=F32)
            for b in range(C // 16):
                l0 = u * C + b * 16
                rr = pl.ds(r0 + l0, 16)
                x = q_v[rr, :].astype(F32)
                kv = v_v[rr, :].astype(F32)
                h = _ln(x) * (1.0 + ca) + sa
                x = x + ga * (h * (y[b * 16:b * 16 + 16] + kv * sd))
                x_s[l0:l0 + 16, :] = x
                h_s[l0:l0 + 16, :] = (_ln(x) * (1.0 + cb) + sb).astype(BF)

    def ffn(t, x_s, h_s):
        rows = pl.ds(pl.multiple_of(t * TM, TM), TM)
        gb = mod_v[0:1, 5 * D:6 * D]
        h2 = h_s[...]
        x = x_s[...]
        a = jnp.dot(h2, w1t_v[...], preferred_element_type=F32)
        a = a + b1_ref[...].astype(F32).reshape(1, F)
        a = jax.nn.gelu(a, approximate=True).astype(BF)
        o = jnp.dot(a, w2_v[...], preferred_element_type=F32) + b2_ref[...].astype(F32).reshape(1, D)
        o_v[rows, :] = (x + gb * o).astype(BF)

    def p3(u, carry):
        t = 2 * u
        pre(t + 1, x_t, h_t)
        ffn(t, x_s, h_s)
        pre(jnp.minimum(t + 2, S // TM - 1), x_s, h_s)
        ffn(t + 1, x_t, h_t)
        out_copy(t).start()
        out_copy(t + 1).start()
        return carry

    with jax.named_scope("p3"):
        pre(0, x_s, h_s)
        lax.fori_loop(0, S // TM // 2, p3, 0)
    for t in range(S // TM):
        out_copy(t).wait()


@jax.jit
def pallas_adaLN_cond__ssm_conv_h3__dense_activation_gelu__prompt_kernel(
    A_q, A_k, A_v, A_shift_k, A_ssm_k, A_ssm_D, B_x, B_w1, B_b1, B_w2, B_b2, c, w_mod,
):
    del B_x
    wf, wi = _dft_mats()
    any_spec = pl.BlockSpec(memory_space=pl.ANY)
    vm = pl.BlockSpec(memory_space=pltpu.VMEM)
    out = pl.pallas_call(
        _kernel,
        out_shape=jax.ShapeDtypeStruct((S, D), BF),
        in_specs=[any_spec] * 7 + [vm] * 7,
        out_specs=any_spec,
        scratch_shapes=[
            pltpu.VMEM((S, D), BF),
            pltpu.VMEM((S + HALO, D), BF),
            pltpu.VMEM((S, D), BF),
            pltpu.VMEM((D, S), BF),
            pltpu.VMEM((F, D), BF),
            pltpu.VMEM((F, D), BF),
            pltpu.VMEM((D, 6 * D), BF),
            pltpu.VMEM((NC, N, D), F32),
            pltpu.VMEM((NC + 1, N, D), F32),
            pltpu.VMEM((NC, N, D), F32),
            pltpu.VMEM((S, D), BF),
            pltpu.VMEM((8, 6 * D), F32),
            pltpu.VMEM((D, F), BF),
            pltpu.VMEM((TM, D), F32),
            pltpu.VMEM((TM, D), BF),
            pltpu.VMEM((TM, D), F32),
            pltpu.VMEM((TM, D), BF),
            pltpu.SemaphoreType.DMA((3, 4)),
            pltpu.SemaphoreType.DMA((4,)),
            pltpu.SemaphoreType.DMA((S // TM,)),
        ],
        compiler_params=pltpu.CompilerParams(vmem_limit_bytes=110 * 1024 * 1024),
    )(A_q.reshape(S, D), A_k.reshape(S, D), A_v.reshape(S, D), A_ssm_k, B_w1.T, B_w2, w_mod,
      A_shift_k.T, A_ssm_D, B_b1, B_b2, c,
      jnp.asarray(wf, BF), jnp.asarray(wi, BF))
    return out.reshape(1, S, D)
```
